```python
import os as _os
_os.environ.setdefault("JAX_PLATFORMS", "cpu")
import jax
import jax.numpy as jnp

def _softmax(x, axis=-1):
    return jax.nn.softmax(x, axis=axis)
def _gelu(x):
    return jax.nn.gelu(x, approximate=True)
def _silu(x):
    return jax.nn.silu(x)
def _sigmoid(x):
    return jax.nn.sigmoid(x)
def _layernorm(x, axis=-1, eps=1e-5):
    m = jnp.mean(x, axis=axis, keepdims=True)
    v = jnp.var(x, axis=axis, keepdims=True)
    return (x - m) / jnp.sqrt(v + eps)
def _scatter_add(tgt, idx, src, axis=0):
    return tgt.at[idx].add(src)
def _segment_sum(src, seg, n):
    return jax.ops.segment_sum(src, seg, n)
class _Rng:
    def __init__(self, key):
        self._k = key
    def _next(self):
        self._k, sub = jax.random.split(self._k)
        return sub
    def normal(self, shape):
        return jax.random.normal(self._next(), shape, dtype=jnp.bfloat16)
    def randint(self, lo, hi, shape):
        return jax.random.randint(self._next(), shape, lo, hi, dtype=jnp.int32)
    def uniform(self, shape, lo=0.0, hi=1.0):
        return jax.random.uniform(self._next(), shape, jnp.bfloat16, lo, hi)
    def permutation(self, n):
        return jax.random.permutation(self._next(), n)


kernel_name = 'standalone__gqa_block_cached__near_ridge'

def setup_inputs():
    _rng = _Rng(jax.random.key(int.from_bytes(__import__("os").urandom(4), "little")))
    _w = (lambda a: (lambda t: t.astype(jnp.bfloat16) if jnp.issubdtype(t.dtype, jnp.floating) else t)(jnp.asarray(a)))
    B, Sq, D = 16, 128, 576
    Hq, Hkv, Sk, Dh = 32, 16, 1024, 128
    assert Hq % Hkv == 0, (Hq, Hkv)
    return {
        "x": _w((lambda *s: _rng.normal(s) * 0.8)(B, Sq, D)),
        "k_cache": _w((lambda *s: _rng.normal(s) * 0.8)(B, Hkv, Sk, Dh)),
        "v_cache": _w((lambda *s: _rng.normal(s) * 0.05)(B, Hkv, Sk, Dh)),
        "wq": _w((lambda *s: _rng.normal(s) * 0.8)(D, Hq * Dh) * (D ** -0.5)),
        "wo": _w((lambda *s: _rng.normal(s) * 0.05)(Hq * Dh, D) * ((Hq * Dh) ** -0.5)),
    }

def reference(x, k_cache, v_cache, wq, wo):
    B, Sq, D = x.shape
    Hq, Dh = 32, 128
    Hkv = k_cache.shape[1]
    rep = Hq // Hkv
    q = (lambda x, *d: x.transpose(*d))((x @ wq).reshape(B, Sq, Hq, Dh), 0, 2, 1, 3)
    k = jnp.repeat(k_cache, rep, axis=1)
    v = jnp.repeat(v_cache, rep, axis=1)
    scores = jnp.einsum("bhqd,bhkd->bhqk", q, k) * (Dh ** -0.5)
    p = _softmax(scores, axis=-1)
    o = jnp.einsum("bhqk,bhkd->bhqd", p, v)
    return (lambda x, *d: x.transpose(*d))(o, 0, 2, 1, 3).reshape(B, Sq, Hq * Dh) @ wo
```

```python
import functools
import math
import jax
import jax.numpy as jnp
import jax.experimental.pallas as pl
import jax.experimental.pallas.tpu as pltpu

G = 8

def _kernel(xt_ref, k_ref, v_ref, wq_hbm, wot_hbm, o_ref, x_ref, acc_ref, wq_ref, wot_ref, sems, *, G, nhg, scale):
    b = pl.program_id(0)
    hg = pl.program_id(1)
    W = G * 256

    def wq_copy(i):
        return pltpu.make_async_copy(wq_hbm.at[:, pl.ds(i * W, W)], wq_ref.at[:, pl.ds(i * W, W)], sems.at[0, i])

    def wot_copy(i):
        return pltpu.make_async_copy(wot_hbm.at[:, pl.ds(i * W, W)], wot_ref.at[:, pl.ds(i * W, W)], sems.at[1, i])

    @pl.when(jnp.logical_and(b == 0, hg == 0))
    def _():
        for i in range(nhg):
            wq_copy(i).start()
            wot_copy(i).start()

    @pl.when(hg == 0)
    def _():
        acc_ref[...] = jnp.zeros_like(acc_ref)
        x_ref[...] = xt_ref[0].T

    for i in range(nhg):
        @pl.when(jnp.logical_and(b == 0, hg == i))
        def _():
            wq_copy(i).wait()

    x = x_ref[...]
    Sq = x.shape[0]
    col0 = pl.multiple_of(hg * W, 256)
    wq = wq_ref[:, pl.ds(col0, W)]
    q = jnp.dot(x, wq, preferred_element_type=jnp.float32)
    q = (q * scale).astype(jnp.bfloat16)
    outs = []
    nt = (((1,), (1,)), ((), ()))
    for g in range(G):
        k = k_ref[0, g]
        v = v_ref[0, g]
        q2 = jnp.concatenate([q[:, (2*g)*128:(2*g+1)*128], q[:, (2*g+1)*128:(2*g+2)*128]], axis=0)
        s = jax.lax.dot_general(q2, k, nt, preferred_element_type=jnp.float32)
        m = jnp.max(s, axis=-1, keepdims=True)
        p = jnp.exp2(s - m)
        l = jnp.sum(p, axis=-1, keepdims=True)
        o = jnp.dot(p.astype(jnp.bfloat16), v, preferred_element_type=jnp.float32)
        o = (o / l).astype(jnp.bfloat16)
        outs.append(o[:Sq])
        outs.append(o[Sq:])
    ocat = jnp.concatenate(outs, axis=1)

    for i in range(nhg):
        @pl.when(jnp.logical_and(b == 0, hg == i))
        def _():
            wot_copy(i).wait()

    wot = wot_ref[:, pl.ds(col0, W)]
    acc_ref[...] += jax.lax.dot_general(wot, ocat, nt, preferred_element_type=jnp.float32)

    @pl.when(hg == nhg - 1)
    def _():
        o_ref[0] = acc_ref[...].astype(o_ref.dtype)


@jax.jit
def pallas_standalone__gqa_block_cached__near_ridge_kernel(x, k_cache, v_cache, wq, wo):
    B, Sq, D = x.shape
    _, Hkv, Sk, Dh = k_cache.shape
    HqDh = wq.shape[1]
    nhg = Hkv // G
    scale = Dh ** -0.5 * math.log2(math.e)
    kern = functools.partial(_kernel, G=G, nhg=nhg, scale=scale)
    xt = jnp.swapaxes(x, 1, 2)
    wot = wo.T
    out_t = pl.pallas_call(
        kern,
        grid=(B, nhg),
        in_specs=[
            pl.BlockSpec((1, D, Sq), lambda b, h: (b, 0, 0)),
            pl.BlockSpec((1, G, Sk, Dh), lambda b, h: (b, h, 0, 0)),
            pl.BlockSpec((1, G, Sk, Dh), lambda b, h: (b, h, 0, 0)),
            pl.BlockSpec(memory_space=pl.ANY),
            pl.BlockSpec(memory_space=pl.ANY),
        ],
        out_specs=pl.BlockSpec((1, D, Sq), lambda b, h: (b, 0, 0)),
        out_shape=jax.ShapeDtypeStruct((B, D, Sq), x.dtype),
        scratch_shapes=[pltpu.VMEM((Sq, D), x.dtype), pltpu.VMEM((D, Sq), jnp.float32),
                        pltpu.VMEM((D, HqDh), wq.dtype), pltpu.VMEM((D, HqDh), wo.dtype),
                        pltpu.SemaphoreType.DMA((2, nhg))],
        compiler_params=pltpu.CompilerParams(
            dimension_semantics=("arbitrary", "arbitrary"),
            vmem_limit_bytes=100 * 1024 * 1024,
        ),
    )(xt, k_cache, v_cache, wq, wot)
    return jnp.swapaxes(out_t, 1, 2)
```

```python
import functools
import math
import jax
import jax.numpy as jnp
import jax.experimental.pallas as pl
import jax.experimental.pallas.tpu as pltpu

G = 8


def _kernel(xt_ref, k_ref, v_ref, wq_hbm, wot_hbm, o_ref, x_ref, q_ref, acc_ref, wq_ref, wot_ref, sems, *, G, nhg, scale):
    b = pl.program_id(0)
    hg = pl.program_id(1)
    W = G * 256
    nt = (((1,), (1,)), ((), ()))

    def wq_copy(i):
        return pltpu.make_async_copy(wq_hbm.at[:, pl.ds(i * W, W)], wq_ref.at[:, pl.ds(i * W, W)], sems.at[0, i])

    def wot_copy(i):
        return pltpu.make_async_copy(wot_hbm.at[:, pl.ds(i * W, W)], wot_ref.at[:, pl.ds(i * W, W)], sems.at[1, i])

    def qproj(col):
        q = jnp.dot(x_ref[...], wq_ref[:, pl.ds(col, W)], preferred_element_type=jnp.float32)
        return (q * scale).astype(jnp.bfloat16)

    first = jnp.logical_and(b == 0, hg == 0)

    @pl.when(jnp.logical_or(first, hg == nhg - 1))
    def _():
        x_ref[...] = xt_ref[0].T

    @pl.when(first)
    def _():
        wq_copy(0).start()
        wq_copy(0).wait()
        for i in range(1, nhg):
            wq_copy(i).start()
        for i in range(nhg):
            wot_copy(i).start()
        q_ref[...] = qproj(0)

    @pl.when(hg == 0)
    def _():
        acc_ref[...] = jnp.zeros_like(acc_ref)

    for i in range(1, nhg):
        @pl.when(jnp.logical_and(b == 0, hg == i))
        def _():
            wot_copy(i).wait()
            if i + 1 < nhg:
                wq_copy(i + 1).wait()

    def main(is_first):
        q = q_ref[...]
        Sq = q.shape[0]
        col0 = pl.multiple_of(hg * W, 256)
        coln = pl.multiple_of(jnp.where(hg == nhg - 1, 0, hg + 1) * W, 256)
        outs = []
        qn = None
        for g in range(G):
            k = k_ref[0, g]
            v = v_ref[0, g]
            q2 = jnp.concatenate([q[:, (2*g)*128:(2*g+1)*128], q[:, (2*g+1)*128:(2*g+2)*128]], axis=0)
            s = jax.lax.dot_general(q2, k, nt, preferred_element_type=jnp.float32)
            if g == G - 1:
                if is_first and nhg > 1:
                    wq_copy(1).wait()
                qn = qproj(coln)
            m = jnp.max(s, axis=-1, keepdims=True)
            p = jnp.exp2(s - m)
            l = jnp.sum(p, axis=-1, keepdims=True)
            o = jnp.dot(p.astype(jnp.bfloat16), v, preferred_element_type=jnp.float32)
            o = (o / l).astype(jnp.bfloat16)
            outs.append(o[:Sq])
            outs.append(o[Sq:])
        q_ref[...] = qn
        if is_first:
            wot_copy(0).wait()
        ocat = jnp.concatenate(outs, axis=1)
        wot = wot_ref[:, pl.ds(col0, W)]
        acc_ref[...] += jax.lax.dot_general(wot, ocat, nt, preferred_element_type=jnp.float32)

    @pl.when(first)
    def _():
        main(True)

    @pl.when(jnp.logical_not(first))
    def _():
        main(False)

    @pl.when(hg == nhg - 1)
    def _():
        o_ref[0] = acc_ref[...].astype(o_ref.dtype)


@jax.jit
def pallas_standalone__gqa_block_cached__near_ridge_kernel(x, k_cache, v_cache, wq, wo):
    B, Sq, D = x.shape
    _, Hkv, Sk, Dh = k_cache.shape
    HqDh = wq.shape[1]
    nhg = Hkv // G
    scale = Dh ** -0.5 * math.log2(math.e)
    kern = functools.partial(_kernel, G=G, nhg=nhg, scale=scale)
    xt = jnp.swapaxes(x, 1, 2)
    wot = wo.T

    def x_map(b, h):
        return (jnp.minimum(b + (h + 1) // nhg, B - 1), 0, 0)

    out_t = pl.pallas_call(
        kern,
        grid=(B, nhg),
        in_specs=[
            pl.BlockSpec((1, D, Sq), x_map),
            pl.BlockSpec((1, G, Sk, Dh), lambda b, h: (b, h, 0, 0)),
            pl.BlockSpec((1, G, Sk, Dh), lambda b, h: (b, h, 0, 0)),
            pl.BlockSpec(memory_space=pl.ANY),
            pl.BlockSpec(memory_space=pl.ANY),
        ],
        out_specs=pl.BlockSpec((1, D, Sq), lambda b, h: (b, 0, 0)),
        out_shape=jax.ShapeDtypeStruct((B, D, Sq), x.dtype),
        scratch_shapes=[pltpu.VMEM((Sq, D), x.dtype), pltpu.VMEM((Sq, G * 256), x.dtype),
                        pltpu.VMEM((D, Sq), jnp.float32),
                        pltpu.VMEM((D, HqDh), wq.dtype), pltpu.VMEM((D, HqDh), wo.dtype),
                        pltpu.SemaphoreType.DMA((2, nhg))],
        compiler_params=pltpu.CompilerParams(
            dimension_semantics=("arbitrary", "arbitrary"),
            vmem_limit_bytes=100 * 1024 * 1024,
        ),
    )(xt, k_cache, v_cache, wq, wot)
    return jnp.swapaxes(out_t, 1, 2)
```
